```python
import os as _os
_os.environ.setdefault('JAX_PLATFORMS', 'cpu')
import jax
import jax.numpy as jnp

def _softmax(x, axis=-1):
    return jax.nn.softmax(x, axis=axis)

def _gelu(x):
    return jax.nn.gelu(x, approximate=True)

def _silu(x):
    return jax.nn.silu(x)

def _sigmoid(x):
    return jax.nn.sigmoid(x)

def _layernorm(x, axis=-1, eps=1e-05):
    m = jnp.mean(x, axis=axis, keepdims=True)
    v = jnp.var(x, axis=axis, keepdims=True)
    return (x - m) / jnp.sqrt(v + eps)

def _scatter_add(tgt, idx, src, axis=0):
    return tgt.at[idx].add(src)

def _segment_sum(src, seg, n):
    return jax.ops.segment_sum(src, seg, n)

class _Rng:

    def __init__(self, key):
        self._k = key

    def _next(self):
        self._k, sub = jax.random.split(self._k)
        return sub

    def normal(self, shape):
        return jax.random.normal(self._next(), shape, dtype=jnp.bfloat16)

    def randint(self, lo, hi, shape):
        return jax.random.randint(self._next(), shape, lo, hi, dtype=jnp.int32)

    def uniform(self, shape, lo=0.0, hi=1.0):
        return jax.random.uniform(self._next(), shape, jnp.bfloat16, lo, hi)

    def permutation(self, n):
        return jax.random.permutation(self._next(), n)
kernel_name = 'parallel_sum__memory_aug_recurrent_mem_tr__dense_activation_gelu__prompt'

def setup_inputs():
    _rng = _Rng(jax.random.key(int.from_bytes(__import__("os").urandom(4), "little")))
    _w = lambda a: (lambda t: t.astype(jnp.bfloat16) if jnp.issubdtype(t.dtype, jnp.floating) else t)(jnp.asarray(a))

    def _A_setup():
        B, S, Dm = (1, 2048, 1024)
        H, Dh = (32, 128)
        M, seg = (8, 32)
        seg = min(seg, S)
        S = S // seg * seg
        return {'x': _w((lambda *s: _rng.normal(s) * 0.05)(B, S, Dm)), 'mem0': _w((lambda *s: _rng.normal(s) * 0.2)(B, M, Dm)), 'Wq': _w((lambda *s: _rng.normal(s) * 0.8)(Dm, H, Dh) * Dm ** (-0.5)), 'Wk': _w((lambda *s: _rng.normal(s) * 0.8)(Dm, H, Dh) * Dm ** (-0.5)), 'Wv': _w((lambda *s: _rng.normal(s) * 0.2)(Dm, H, Dh) * Dm ** (-0.5)), 'Wo': _w((lambda *s: _rng.normal(s) * 0.2)(H, Dh, Dm) * (H * Dh) ** (-0.5)), 'seg_len': seg}
    _A_in = _A_setup()

    def _B_setup():
        B, S, D, F = (1, 2048, 1024, 3584)
        return {'x': _w((lambda *s: _rng.normal(s) * 0.05)(B, S, D)), 'w1': _w((lambda *s: _rng.normal(s) * 0.1)(D, F) * D ** (-0.5)), 'b1': _w((lambda *s: _rng.normal(s) * 0.1)(F) * 0.01), 'w2': _w((lambda *s: _rng.normal(s) * 0.1)(F, D) * F ** (-0.5)), 'b2': _w((lambda *s: _rng.normal(s) * 0.05)(D) * 0.01)}
    _B_in = _B_setup()
    return {'A_x': _A_in['x'], 'A_mem0': _A_in['mem0'], 'A_Wq': _A_in['Wq'], 'A_Wk': _A_in['Wk'], 'A_Wv': _A_in['Wv'], 'A_Wo': _A_in['Wo'], 'A_seg_len': _A_in['seg_len'], 'B_x': _B_in['x'], 'B_w1': _B_in['w1'], 'B_b1': _B_in['b1'], 'B_w2': _B_in['w2'], 'B_b2': _B_in['b2']}

def reference(A_x, A_mem0, A_Wq, A_Wk, A_Wv, A_Wo, A_seg_len, B_x, B_w1, B_b1, B_w2, B_b2):

    def _A_ref(x, mem0, Wq, Wk, Wv, Wo, seg_len):
        B, S, Dm = x.shape
        H, Dh = (Wq.shape[1], Wq.shape[2])
        M = mem0.shape[1]
        scale = Dh ** (-0.5)
        n_seg = S // seg_len
        L = M + seg_len
        idx = jnp.arange(L)
        mask = (idx[:, None] < M) | (idx[:, None] >= idx[None, :])
        mem = mem0
        outs = []
        for s in range(n_seg):
            xs = x[:, s * seg_len:(s + 1) * seg_len, :].copy()
            h = jnp.concatenate([mem, xs], axis=1)
            q = jnp.einsum('btd,dhe->bhte', h, Wq)
            k = jnp.einsum('btd,dhe->bhte', h, Wk)
            v = jnp.einsum('btd,dhe->bhte', h, Wv)
            scores = jnp.einsum('bhqe,bhke->bhqk', q, k) * scale
            scores = jnp.where(mask[None, None], scores, -1000000000.0)
            p = _softmax(scores, axis=-1)
            o = jnp.einsum('bhqk,bhke->bhqe', p, v)
            o = jnp.einsum('bhte,hed->btd', o, Wo)
            mem = o[:, :M, :].copy()
            outs.append(o[:, M:, :])
        return jnp.concatenate(outs, axis=1)

    def _B_ref(x, w1, b1, w2, b2):
        h = jnp.einsum('bsd,df->bsf', x, w1) + b1
        h = _gelu(h)
        return jnp.einsum('bsf,fd->bsd', h, w2) + b2
    x = A_x
    xn = _layernorm(x, axis=-1)
    return x + _A_ref(xn, A_mem0, A_Wq, A_Wk, A_Wv, A_Wo, A_seg_len) + _B_ref(xn, B_w1, B_b1, B_w2, B_b2)
```

```python
import functools
import math

import jax
import jax.numpy as jnp
import numpy as np
import jax.experimental.pallas as pl
import jax.experimental.pallas.tpu as pltpu

F32 = jnp.float32
BF16 = jnp.bfloat16
U32 = jnp.uint32


def _dot(a, b):
    return jnp.dot(a, b, preferred_element_type=F32)


def _dot_nt(a, b):
    return jax.lax.dot_general(a, b, (((1,), (1,)), ((), ())), preferred_element_type=F32)


def _gelu(x):
    c = np.float32(math.sqrt(2.0 / math.pi))
    return 0.5 * x * (1.0 + jnp.tanh(c * (x + np.float32(0.044715) * (x * x * x))))


def _as_bf16(w_u32):
    return pltpu.bitcast(w_u32, BF16)


@functools.partial(jax.jit, static_argnames=("A_seg_len",))
def pallas_parallel_sum__memory_aug_recurrent_mem_tr__dense_activation_gelu__prompt_kernel(
    A_x: jax.Array,
    A_mem0: jax.Array,
    A_Wq: jax.Array,
    A_Wk: jax.Array,
    A_Wv: jax.Array,
    A_Wo: jax.Array,
    A_seg_len: int,
    B_x: jax.Array,
    B_w1: jax.Array,
    B_b1: jax.Array,
    B_w2: jax.Array,
    B_b2: jax.Array,
):
    del B_x
    _, S, D = A_x.shape
    M = A_mem0.shape[1]
    _, H, DH = A_Wq.shape
    F = B_w1.shape[1]
    SEG = int(A_seg_len)
    NSEG = S // SEG
    L = M + SEG
    scale = np.float32(DH ** (-0.5))

    R = 256
    NB = S // R
    C = 512
    CH = D // NB

    def kernel(x_hbm, mem0_ref, wq_hbm, wk_hbm, wv_hbm, wo_hbm, w1_hbm, b1_ref, w2_hbm, b2_ref,
               out_hbm,
               xs, xn, acc, ob, w1s, w2s, wos, wqkv, stage, hbuf,
               sem_x, sem_w1, sem_w2, sem_wo, sem_st, sem_out):
        w_hbm = (wq_hbm, wk_hbm, wv_hbm)

        def x_copy():
            return pltpu.make_async_copy(x_hbm.at[0], xs, sem_x)

        def w1_copy():
            return pltpu.make_async_copy(w1_hbm, w1s.bitcast(BF16), sem_w1)

        def w2_copy():
            return pltpu.make_async_copy(w2_hbm, w2s.bitcast(BF16), sem_w2)

        def wo_copy():
            return pltpu.make_async_copy(wo_hbm, wos.bitcast(BF16), sem_wo)

        def stage_copy(rb, j):
            slot = rb % 2
            src = w_hbm[j].at[pl.ds(pl.multiple_of(rb * (CH * H), CH * H), CH * H), :]
            return pltpu.make_async_copy(src, stage.at[slot, j], sem_st.at[slot, j])

        def layernorm(rb):
            r0 = pl.multiple_of(rb * R, R)
            x = xs[pl.ds(r0, R), :].astype(F32)
            mean = jnp.mean(x, axis=-1, keepdims=True)
            xc = x - mean
            var = jnp.mean(xc * xc, axis=-1, keepdims=True)
            y = xc * jax.lax.rsqrt(var + np.float32(1e-5))
            xn[pl.ds(r0, R), :] = y.astype(BF16).astype(F32)

        def ffn_up(rb, slot):
            r0 = pl.multiple_of(rb * R, R)
            x = xn[pl.ds(r0, R), :]
            for c in range(F // C):
                w = _as_bf16(w1s[:, c * C:(c + 1) * C])
                b = b1_ref[pl.ds(c * C, C)].astype(F32).reshape(1, C)
                hbuf[slot, :, c * C:(c + 1) * C] = _gelu(_dot(x, w) + b).astype(BF16)

        def ffn_down(rb, slot):
            r0 = pl.multiple_of(rb * R, R)
            y = _dot(hbuf[slot], _as_bf16(w2s[...]))
            b = b2_ref[...].astype(F32).reshape(1, D)
            acc[pl.ds(r0, R), :] = xs[pl.ds(r0, R), :].astype(F32) + (y + b)

        def relayout(rb, j):
            slot = rb % 2
            o0 = pl.multiple_of(rb * (CH // 2), CH // 2)
            w = stage[slot, j].reshape(CH, H, DH)
            wt = jnp.swapaxes(w, 0, 1)
            for h in range(H):
                wqkv[h, j, pl.ds(o0, CH // 2), :] = pltpu.bitcast(wt[h], U32)

        x_copy().start()
        w1_copy().start()
        x_copy().wait()
        w2_copy().start()
        layernorm(0)
        layernorm(1)
        w1_copy().wait()
        for j in range(3):
            stage_copy(0, j).start()
        ffn_up(0, 0)
        w2_copy().wait()
        wo_copy().start()

        def ffn_body(rb, carry):
            slot = rb % 2
            nxt = jnp.minimum(rb + 1, NB - 1)

            @pl.when(rb + 1 < NB)
            def _():
                for j in range(3):
                    stage_copy(rb + 1, j).start()

            for j in range(3):
                stage_copy(rb, j).wait()
            ffn_up(nxt, 1 - slot)
            for j in range(3):
                relayout(rb, j)
            ffn_down(rb, slot)
            layernorm(jnp.minimum(rb + 2, NB - 1))
            return carry

        jax.lax.fori_loop(0, NB, ffn_body, 0)
        wo_copy().wait()

        row = jax.lax.broadcasted_iota(jnp.int32, (L, L), 0)
        col = jax.lax.broadcasted_iota(jnp.int32, (L, L), 1)
        mask = (row < M) | (row >= col)

        def out_copy(s):
            t0 = pl.multiple_of(s * SEG, SEG)
            return pltpu.make_async_copy(ob.at[pl.ds(t0, SEG), :],
                                         out_hbm.at[0, pl.ds(t0, SEG), :], sem_out)

        def step(s, mem):
            t0 = pl.multiple_of(s * SEG, SEG)
            hx = jnp.concatenate([mem, xn[pl.ds(t0, SEG), :]], axis=0)
            q, kb, vb, e, l, o = {}, {}, {}, {}, {}, {}
            y = [None] * (D // 128)
            for i in range(H + 3):
                if 0 <= i - 1 < H:
                    sc = _dot_nt(q[i - 1], kb[i - 1])
                if i < H:
                    q[i] = _dot(hx, _as_bf16(wqkv[i, 0]))
                if 0 <= i - 1 < H:
                    sc = jnp.where(mask, sc * scale, np.float32(-1e9))
                    m = jnp.max(sc, axis=-1, keepdims=True)
                    e[i - 1] = jnp.exp(sc - m)
                    l[i - 1] = jnp.sum(e[i - 1], axis=-1, keepdims=True)
                if i < H:
                    kb[i] = _dot(hx, _as_bf16(wqkv[i, 1])).astype(BF16)
                if 0 <= i - 2 < H:
                    o[i - 2] = _dot(e[i - 2], vb[i - 2]) / l[i - 2]
                if i < H:
                    vb[i] = _dot(hx, _as_bf16(wqkv[i, 2])).astype(BF16)
                if 0 <= i - 3 < H:
                    h = i - 3
                    for c in range(D // 128):
                        t = _dot(o[h], _as_bf16(wos[h, :, c * 128:(c + 1) * 128]))
                        y[c] = t if y[c] is None else y[c] + t
            yv = jnp.concatenate(y, axis=1)
            ob[pl.ds(t0, SEG), :] = (acc[pl.ds(t0, SEG), :] + yv[M:]).astype(BF16)
            out_copy(s).start()
            return yv[:M]

        jax.lax.fori_loop(0, NSEG, step, mem0_ref[0].astype(F32))
        pltpu.make_async_copy(ob, out_hbm.at[0], sem_out).wait()

    hbm = pl.BlockSpec(memory_space=pl.ANY)
    vmem = pl.BlockSpec(memory_space=pltpu.VMEM)
    return pl.pallas_call(
        kernel,
        out_shape=jax.ShapeDtypeStruct(A_x.shape, A_x.dtype),
        in_specs=[hbm, vmem, hbm, hbm, hbm, hbm, hbm, vmem, hbm, vmem],
        out_specs=hbm,
        scratch_shapes=[
            pltpu.VMEM((S, D), BF16),
            pltpu.VMEM((S, D), F32),
            pltpu.VMEM((S, D), F32),
            pltpu.VMEM((S, D), BF16),
            pltpu.VMEM((D // 2, F), U32),
            pltpu.VMEM((F // 2, D), U32),
            pltpu.VMEM((H, DH // 2, D), U32),
            pltpu.VMEM((H, 3, D // 2, DH), U32),
            pltpu.VMEM((2, 3, CH * H, DH), BF16),
            pltpu.VMEM((2, R, F), BF16),
            pltpu.SemaphoreType.DMA(()),
            pltpu.SemaphoreType.DMA(()),
            pltpu.SemaphoreType.DMA(()),
            pltpu.SemaphoreType.DMA(()),
            pltpu.SemaphoreType.DMA((2, 3)),
            pltpu.SemaphoreType.DMA(()),
        ],
        compiler_params=pltpu.CompilerParams(vmem_limit_bytes=110 * 1024 * 1024),
    )(A_x, A_mem0, A_Wq.reshape(D * H, DH), A_Wk.reshape(D * H, DH), A_Wv.reshape(D * H, DH),
      A_Wo, B_w1, B_b1, B_w2, B_b2)
```

```python
import functools
import math

import jax
import jax.numpy as jnp
import numpy as np
import jax.experimental.pallas as pl
import jax.experimental.pallas.tpu as pltpu

F32 = jnp.float32
BF16 = jnp.bfloat16
U32 = jnp.uint32

CFG = dict(
    R=256,
    MS=128,
    WC=512,
    ln_rows=32,
    defer=0,
    nsteps=None,
    scopes=False,
)


def _scope(name):
    import contextlib
    return jax.named_scope(name) if CFG["scopes"] else contextlib.nullcontext()


def _dot(a, b):
    return jnp.dot(a, b, preferred_element_type=F32)


def _dot_nt(a, b):
    return jax.lax.dot_general(a, b, (((1,), (1,)), ((), ())), preferred_element_type=F32)


def _gelu(x):
    c = np.float32(math.sqrt(2.0 / math.pi))
    return 0.5 * x * (1.0 + jnp.tanh(c * (x + np.float32(0.044715) * (x * x * x))))


def _as_bf16(w_u32):
    return pltpu.bitcast(w_u32, BF16)


def _transpose8(e):
    s = jax.lax.broadcasted_iota(jnp.int32, (1, 8, 128), 1)
    for k in (4, 2, 1):
        x = e.reshape(8 // (2 * k), 2, k, 8, 128)
        a = x[:, 0].reshape(4, 8, 128)
        b = x[:, 1].reshape(4, 8, 128)
        m = (s & k) == 0
        na = jnp.where(m, a, pltpu.roll(b, k, 1)).reshape(8 // (2 * k), 1, k, 8, 128)
        nb = jnp.where(m, pltpu.roll(a, 8 - k, 1), b).reshape(8 // (2 * k), 1, k, 8, 128)
        e = jnp.concatenate([na, nb], axis=1).reshape(8, 8, 128)
    return e


def _kernel_impl(A_x, A_mem0, A_Wq, A_Wk, A_Wv, A_Wo, A_seg_len, B_x, B_w1, B_b1, B_w2, B_b2):
    del B_x
    _, S, D = A_x.shape
    M = A_mem0.shape[1]
    _, H, DH = A_Wq.shape
    F = B_w1.shape[1]
    SEG = int(A_seg_len)
    NSEG = S // SEG
    L = M + SEG
    scale = np.float32(DH ** (-0.5))

    R = CFG["R"]
    MS = CFG["MS"]
    WC = CFG["WC"]
    NB = S // R
    NIT = NB - 2
    ND = D // 128
    NT = F // 128
    NWC = F // WC
    CH = -(-D // (16 * NIT)) * 16
    DEFER = CFG["defer"]

    H_OFF = 0
    ST_OFF = H_OFF + 2 * NT * (R // 2)
    ST_ROWS = CH * (H // 2)
    WQ_OFF = ST_OFF + 2 * 3 * ST_ROWS
    WA_ROWS = WQ_OFF + H * 3 * (D // 2)
    ACC_OFF = 0
    X_OFF = ACC_OFF + ND * S
    WB_ROWS = X_OFF + ND * (S // 2)

    def kernel(x_hbm, mem0_ref, wq_hbm, wk_hbm, wv_hbm, wo_hbm, w1_hbm, b1_ref, w2_hbm, b2_ref,
               out_hbm,
               wa, wb, xn, ob, w1s, w2s, wos, b1f,
               sem_x, sem_w1, sem_w2, sem_wo, sem_st, sem_out):
        w_hbm = (wq_hbm, wk_hbm, wv_hbm)

        def ds(start, size, align=8):
            if isinstance(start, int):
                return pl.ds(start, size)
            return pl.ds(pl.multiple_of(start, align), size)

        def x_copies(rb):
            return [pltpu.make_async_copy(
                x_hbm.at[0, ds(rb * R, R, R), pl.ds(c * 128, 128)],
                wb.at[ds(X_OFF + c * (S // 2) + rb * (R // 2), R // 2), :].bitcast(BF16),
                sem_x.at[rb]) for c in range(ND)]

        def x_start(rb):
            for cp in x_copies(rb):
                cp.start()

        def x_wait(rb):
            for cp in x_copies(rb):
                cp.wait()

        def w1_copy(c):
            return pltpu.make_async_copy(w1_hbm.at[:, ds(c * WC, WC, WC)],
                                         w1s.bitcast(BF16).at[:, ds(c * WC, WC, WC)], sem_w1.at[c])

        def w2_copy():
            return pltpu.make_async_copy(w2_hbm, w2s.bitcast(BF16), sem_w2)

        def wo_copy():
            return pltpu.make_async_copy(wo_hbm, wos.bitcast(BF16), sem_wo)

        def group_row0(g):
            if isinstance(g, int):
                return min(g * CH, D - CH)
            return pl.multiple_of(jnp.minimum(g * CH, D - CH), 16)

        def stage_copy(g, j):
            slot = g % 2
            src = w_hbm[j].at[ds(group_row0(g) * H, CH * H), :]
            dst = wa.at[ds(ST_OFF + (slot * 3 + j) * ST_ROWS, ST_ROWS), :].bitcast(BF16)
            return pltpu.make_async_copy(src, dst, sem_st.at[slot, j])

        def stage_start(g):
            for j in range(3):
                stage_copy(g, j).start()

        def stage_wait(g):
            for j in range(3):
                stage_copy(g, j).wait()

        def load_x(r0, n, c):
            w = wb[ds(X_OFF + c * (S // 2) + r0 // 2, n // 2), :]
            return _as_bf16(w).astype(F32)

        def layernorm(r0, n):
            x = jnp.concatenate([load_x(r0, n, c) for c in range(ND)], axis=1)
            mean = jnp.mean(x, axis=-1, keepdims=True)
            xc = x - mean
            var = jnp.mean(xc * xc, axis=-1, keepdims=True)
            y = xc * jax.lax.rsqrt(var + np.float32(1e-5))
            xn[ds(r0, n), :] = y.astype(BF16).astype(F32)

        def h_rows(slot, t, m0):
            return ds(H_OFF + (slot * NT + t) * (R // 2) + m0 // 2, MS // 2)

        def ffn_up(rb, m0, t):
            w = _as_bf16(w1s[:, ds(t * 128, 128, 128)])
            b = b1f[0:1, ds(t * 128, 128, 128)]
            h = _gelu(_dot(xn[ds(rb * R + m0, MS), :], w) + b)
            wa[h_rows(rb % 2, t, m0), :] = pltpu.bitcast(h.astype(BF16), U32)

        def ffn_down(rb, m0, c):
            h = _as_bf16(jnp.concatenate([wa[h_rows(rb % 2, t, m0), :] for t in range(NT)], axis=1))
            y = _dot(h, _as_bf16(w2s[:, c * 128:(c + 1) * 128]))
            b = b2_ref[pl.ds(c * 128, 128)].astype(F32).reshape(1, 128)
            r0 = rb * R + m0
            wb[ds(ACC_OFF + c * S + r0, MS), :] = pltpu.bitcast(load_x(r0, MS, c) + (y + b), U32)

        def relayout(g, j, p, half):
            slot = g % 2
            x = wa[ds(ST_OFF + (slot * 3 + j) * ST_ROWS + p * 16 * (H // 2), 16 * (H // 2)), :]
            x = x.reshape(8, 2, H // 16, 8, 128)[:, :, half]
            a, b = x[:, 0], x[:, 1]
            even = pltpu.pack_elementwise([a, b], packed_dtype=jnp.uint16)
            odd = pltpu.pack_elementwise(
                [pltpu.unpack_elementwise(v, index=1, packed_dtype=jnp.uint16, unpacked_dtype=U32)
                 for v in (a, b)], packed_dtype=jnp.uint16)
            o0 = group_row0(g) // 2 + p * 8
            for par, tt in enumerate((_transpose8(even), _transpose8(odd))):
                for i in range(8):
                    h = 2 * (half * 8 + i) + par
                    wa[ds(WQ_OFF + (h * 3 + j) * (D // 2) + o0, 8), :] = tt[i]

        def interleave(work, pieces, spare=1):
            done = 0
            for i, w in enumerate(work):
                w()
                upto = min(((i + 1) * len(pieces)) // max(len(work) - spare, 1), len(pieces))
                while done < upto:
                    pieces[done]()
                    done += 1

        P = functools.partial

        with _scope("p0_first"):
            x_start(0)
            x_start(1)
            for c in range(NWC):
                w1_copy(c).start()
            x_start(2)
            w2_copy().start()
            x_start(3)
            stage_start(0)
            for rb in range(4, NB):
                x_start(rb)
            stage_start(1)
            wo_copy().start()
            b1f[...] = jnp.broadcast_to(b1_ref[...].astype(F32).reshape(1, F), (8, F))
            for rb in range(2):
                x_wait(rb)
                for r0 in range(rb * R, (rb + 1) * R, MS):
                    layernorm(r0, MS)

        def up01_body(c, carry):
            w1_copy(c).wait()
            for tt in range(WC // 128):
                for rb in range(2):
                    for m0 in range(0, R, MS):
                        ffn_up(rb, m0, c * (WC // 128) + tt)
            return carry

        with _scope("p1_up01"):
            jax.lax.fori_loop(0, NWC, up01_body, 0)
        with _scope("p2_mid"):
            w2_copy().wait()

        def ffn_body(rb, carry):
            LNR = CFG["ln_rows"]
            x_wait(rb + 2)
            interleave([P(ffn_down, rb, m0, c) for c in range(ND) for m0 in range(0, R, MS)],
                       [P(layernorm, (rb + 2) * R + r, LNR) for r in range(0, R, LNR)])
            stage_wait(rb)
            interleave([P(ffn_up, rb + 2, m0, t) for t in range(NT) for m0 in range(0, R, MS)],
                       [P(relayout, rb, j, p, half) for j in range(3) for p in range(CH // 16)
                        for half in range(H // 16)])

            @pl.when(rb + 2 < NIT)
            def _():
                stage_start(rb + 2)

            return carry

        def tail_body(rb, carry):
            for c in range(ND):
                for m0 in range(0, R, MS):
                    ffn_down(rb, m0, c)
            return carry

        with _scope("p3_ffn_loop"):
            jax.lax.fori_loop(0, NIT, ffn_body, 0)
        with _scope("p4_ffn_tail"):
            jax.lax.fori_loop(NB - 2, NB, tail_body, 0)
            wo_copy().wait()

        row = jax.lax.broadcasted_iota(jnp.int32, (L, L), 0)
        col = jax.lax.broadcasted_iota(jnp.int32, (L, L), 1)
        mask = (row < M) | (row >= col)

        def w_head(h, j):
            return _as_bf16(wa[pl.ds(WQ_OFF + (h * 3 + j) * (D // 2), D // 2), :])

        def out_copy(s):
            t0 = pl.multiple_of(s * SEG, SEG)
            return pltpu.make_async_copy(ob.at[pl.ds(t0, SEG), :],
                                         out_hbm.at[0, pl.ds(t0, SEG), :], sem_out)

        def step(s, mem):
            t0 = pl.multiple_of(s * SEG, SEG)
            hx = jnp.concatenate([mem, xn[pl.ds(t0, SEG), :]], axis=0)
            q, kb, vb, sc, e, l, o = {}, {}, {}, {}, {}, {}, {}
            y = [None] * (D // 128)

            def scores(h):
                sc[h] = _dot_nt(q[h], kb[h])

            def softmax(h):
                t = jnp.where(mask, sc[h] * scale, np.float32(-1e9))
                m = jnp.max(t, axis=-1, keepdims=True)
                e[h] = jnp.exp(t - m)
                l[h] = jnp.sum(e[h], axis=-1, keepdims=True)

            def pv(h):
                o[h] = _dot(e[h], vb[h]) / l[h]

            def oproj(h):
                for c in range(D // 128):
                    t = _dot(o[h], _as_bf16(wos[h, :, c * 128:(c + 1) * 128]))
                    y[c] = t if y[c] is None else y[c] + t

            HM = H - DEFER
            for i in range(H):
                if i >= 1:
                    scores(i - 1)
                q[i] = _dot(hx, w_head(i, 0))
                if i >= 1:
                    softmax(i - 1)
                kb[i] = _dot(hx, w_head(i, 1)).astype(BF16)
                if i >= 2:
                    pv(i - 2)
                vb[i] = _dot(hx, w_head(i, 2)).astype(BF16)
                if 0 <= i - 3 < HM:
                    oproj(i - 3)
            rest = list(range(max(min(H - 3, HM), 0), H))
            tail = CFG.get("tail")
            if tail is None:
                scores(H - 1)
                softmax(H - 1)
                pv(H - 2)
                while len(rest) > 2:
                    oproj(rest.pop(0))
                pv(H - 1)
                while rest:
                    oproj(rest.pop(0))
            else:
                n1, n2, n3 = tail
                for _ in range(n1):
                    oproj(rest.pop(0))
                scores(H - 1)
                softmax(H - 1)
                for _ in range(n2):
                    oproj(rest.pop(0))
                pv(H - 2)
                for _ in range(n3):
                    oproj(rest.pop(0))
                pv(H - 1)
                while rest:
                    oproj(rest.pop(0))
            yv = jnp.concatenate(y, axis=1)
            res = jnp.concatenate(
                [pltpu.bitcast(wb[ds(ACC_OFF + c * S + t0, SEG), :], F32) for c in range(ND)], axis=1)
            ob[pl.ds(t0, SEG), :] = (res + yv[M:]).astype(BF16)
            out_copy(s).start()
            return yv[:M]

        with _scope("p5_chain"):
            jax.lax.fori_loop(0, NSEG if CFG["nsteps"] is None else CFG["nsteps"], step,
                              mem0_ref[0].astype(F32))
        if CFG["nsteps"] is None:
            pltpu.make_async_copy(ob, out_hbm.at[0], sem_out).wait()
        elif CFG["nsteps"] > 0:
            n = CFG["nsteps"] * SEG
            pltpu.make_async_copy(ob.at[pl.ds(0, n)], out_hbm.at[0, pl.ds(0, n)], sem_out).wait()

    hbm = pl.BlockSpec(memory_space=pl.ANY)
    vmem = pl.BlockSpec(memory_space=pltpu.VMEM)
    return pl.pallas_call(
        kernel,
        out_shape=jax.ShapeDtypeStruct(A_x.shape, A_x.dtype),
        in_specs=[hbm, vmem, hbm, hbm, hbm, hbm, hbm, vmem, hbm, vmem],
        out_specs=hbm,
        scratch_shapes=[
            pltpu.VMEM((WA_ROWS, 128), U32),
            pltpu.VMEM((WB_ROWS, 128), U32),
            pltpu.VMEM((S, D), F32),
            pltpu.VMEM((S, D), BF16),
            pltpu.VMEM((D // 2, F), U32),
            pltpu.VMEM((F // 2, D), U32),
            pltpu.VMEM((H, DH // 2, D), U32),
            pltpu.VMEM((8, F), F32),
            pltpu.SemaphoreType.DMA((NB,)),
            pltpu.SemaphoreType.DMA((NWC,)),
            pltpu.SemaphoreType.DMA(()),
            pltpu.SemaphoreType.DMA(()),
            pltpu.SemaphoreType.DMA((2, 3)),
            pltpu.SemaphoreType.DMA(()),
        ],
        compiler_params=pltpu.CompilerParams(vmem_limit_bytes=110 * 1024 * 1024),
    )(A_x, A_mem0, A_Wq.reshape(D * H, DH), A_Wk.reshape(D * H, DH), A_Wv.reshape(D * H, DH),
      A_Wo, B_w1, B_b1, B_w2, B_b2)


@functools.partial(jax.jit, static_argnames=("A_seg_len",))
def pallas_parallel_sum__memory_aug_recurrent_mem_tr__dense_activation_gelu__prompt_kernel(
    A_x: jax.Array,
    A_mem0: jax.Array,
    A_Wq: jax.Array,
    A_Wk: jax.Array,
    A_Wv: jax.Array,
    A_Wo: jax.Array,
    A_seg_len: int,
    B_x: jax.Array,
    B_w1: jax.Array,
    B_b1: jax.Array,
    B_w2: jax.Array,
    B_b2: jax.Array,
):
    return _kernel_impl(A_x, A_mem0, A_Wq, A_Wk, A_Wv, A_Wo, A_seg_len, B_x, B_w1, B_b1, B_w2, B_b2)
```

```python
import functools
import math

import jax
import jax.numpy as jnp
import numpy as np
import jax.experimental.pallas as pl
import jax.experimental.pallas.tpu as pltpu

F32 = jnp.float32
BF16 = jnp.bfloat16
U32 = jnp.uint32

ROW_BLOCK = 256
UP_ROWS = 64
DOWN_ROWS = 128
LN_ROWS = 32
START_TILES = 4
HEAD_GROUP = 2
STEP_UNROLL = 2
SLOT_ORDER = ("q", "k", "scores", "softmax", "v", "pv", "out")
LAG_SCORES, LAG_PV, LAG_OUT = 1, 3, 4


def _dot(a, b):
    return jnp.dot(a, b, preferred_element_type=F32)


def _dot_nt(a, b):
    return jax.lax.dot_general(a, b, (((1,), (1,)), ((), ())), preferred_element_type=F32)


def _gelu(x):
    c = np.float32(math.sqrt(2.0 / math.pi))
    return 0.5 * x * (1.0 + jnp.tanh(c * (x + np.float32(0.044715) * (x * x * x))))


def _as_bf16(w):
    return pltpu.bitcast(w, BF16)


def _transpose8(e):
    s = jax.lax.broadcasted_iota(jnp.int32, (1, 8, 128), 1)
    for k in (4, 2, 1):
        x = e.reshape(8 // (2 * k), 2, k, 8, 128)
        a = x[:, 0].reshape(4, 8, 128)
        b = x[:, 1].reshape(4, 8, 128)
        keep = (s & k) == 0
        na = jnp.where(keep, a, pltpu.roll(b, k, 1)).reshape(8 // (2 * k), 1, k, 8, 128)
        nb = jnp.where(keep, pltpu.roll(a, 8 - k, 1), b).reshape(8 // (2 * k), 1, k, 8, 128)
        e = jnp.concatenate([na, nb], axis=1).reshape(8, 8, 128)
    return e


def _ds(start, size, align=8):
    if isinstance(start, int):
        return pl.ds(start, size)
    return pl.ds(pl.multiple_of(start, align), size)


def _interleave(work, pieces):
    done = 0
    for i, w in enumerate(work):
        w()
        upto = min(((i + 1) * len(pieces)) // max(len(work) - 1, 1), len(pieces))
        while done < upto:
            pieces[done]()
            done += 1


@functools.partial(jax.jit, static_argnames=("A_seg_len",))
def pallas_parallel_sum__memory_aug_recurrent_mem_tr__dense_activation_gelu__prompt_kernel(
    A_x: jax.Array,
    A_mem0: jax.Array,
    A_Wq: jax.Array,
    A_Wk: jax.Array,
    A_Wv: jax.Array,
    A_Wo: jax.Array,
    A_seg_len: int,
    B_x: jax.Array,
    B_w1: jax.Array,
    B_b1: jax.Array,
    B_w2: jax.Array,
    B_b2: jax.Array,
):
    del B_x
    _, S, D = A_x.shape
    M = A_mem0.shape[1]
    _, H, DH = A_Wq.shape
    F = B_w1.shape[1]
    SEG = int(A_seg_len)
    NSEG = S // SEG
    L = M + SEG
    scale = np.float32(DH ** (-0.5))

    R, MU, MD, TPI, G = ROW_BLOCK, UP_ROWS, DOWN_ROWS, START_TILES, HEAD_GROUP
    NB = S // R
    NIT = NB - 2
    ND = D // 128
    NT = F // 128
    NG = H // G
    CH = -(-D // (16 * NIT)) * 16
    assert DH == 128 and H % 16 == 0 and H % G == 0 and G * L <= 128
    assert M % 8 == 0 and SEG % 16 == 0 and NSEG % STEP_UNROLL == 0
    assert S % R == 0 and NB >= 4 and NT % TPI == 0 and D % 128 == 0 and F % 128 == 0

    ST_ROWS = CH * (H // 2)
    H_OFF = 0
    ST_OFF = H_OFF + 2 * NT * (R // 2)
    WQ_OFF = ST_OFF + 2 * 3 * ST_ROWS
    WA_ROWS = WQ_OFF + H * 3 * (D // 2)
    ACC_OFF = 0
    X_OFF = ACC_OFF + ND * S
    WB_ROWS = X_OFF + ND * (S // 2)

    def kernel(x_hbm, mem0_hbm, wq_hbm, wk_hbm, wv_hbm, wo_hbm, w1_hbm, b1_hbm, w2_hbm, b2_hbm,
               out_hbm,
               wa, wb, xn, ob, w1s, w2s, wos, b1f, b1v, b2v, mem0v,
               sem_x, sem_w1, sem_w2, sem_wo, sem_st, sem_out, sem_small):
        w_hbm = (wq_hbm, wk_hbm, wv_hbm)
        P = functools.partial

        XG = ((0, R), (R, R), (2 * R, R), (3 * R, S - 3 * R))

        def x_copy(g, c):
            r0, n = XG[g]
            return pltpu.make_async_copy(
                x_hbm.at[0, pl.ds(r0, n), _ds(c * 128, 128, 128)],
                wb.at[_ds(X_OFF + c * (S // 2) + r0 // 2, n // 2), :].bitcast(BF16),
                sem_x.at[g])

        def x_wait(g):
            for c in range(ND):
                x_copy(g, c).wait()

        def w1_copy(t):
            return pltpu.make_async_copy(
                w1_hbm.at[:, _ds(t * 128, 128, 128)],
                w1s.at[_ds(t * (D // 2), D // 2, D // 2), :].bitcast(BF16),
                sem_w1.at[t // TPI])

        def small_copies():
            return (pltpu.make_async_copy(b1_hbm, b1v, sem_small.at[0]),
                    pltpu.make_async_copy(b2_hbm, b2v, sem_small.at[1]),
                    pltpu.make_async_copy(mem0_hbm, mem0v, sem_small.at[2]))

        def w2_copy(_=None):
            return pltpu.make_async_copy(w2_hbm, w2s.bitcast(BF16), sem_w2)

        def wo_copy(_=None):
            return pltpu.make_async_copy(wo_hbm, wos.bitcast(BF16), sem_wo)

        def group_row0(g):
            if isinstance(g, int):
                return min(g * CH, D - CH)
            return pl.multiple_of(jnp.minimum(g * CH, D - CH), 16)

        def stage_copy(g, j, _=None):
            slot = g % 2
            return pltpu.make_async_copy(
                w_hbm[j].at[_ds(group_row0(g) * H, CH * H), :],
                wa.at[_ds(ST_OFF + (slot * 3 + j) * ST_ROWS, ST_ROWS), :].bitcast(BF16),
                sem_st.at[slot, j])

        def out_copy(t0):
            return pltpu.make_async_copy(
                ob.at[pl.ds(t0, SEG), :], out_hbm.at[0, pl.ds(t0, SEG), :], sem_out)

        def start_each(n, make_copy):
            def body(i, carry):
                make_copy(i).start()
                return carry
            jax.lax.fori_loop(0, n, body, 0)

        def load_x(r0, n, c):
            return _as_bf16(wb[_ds(X_OFF + c * (S // 2) + r0 // 2, n // 2), :]).astype(F32)

        def layernorm(r0, n):
            x = jnp.concatenate([load_x(r0, n, c) for c in range(ND)], axis=1)
            mean = jnp.mean(x, axis=-1, keepdims=True)
            xc = x - mean
            var = jnp.mean(xc * xc, axis=-1, keepdims=True)
            y = xc * jax.lax.rsqrt(var + np.float32(1e-5))
            xn[_ds(r0, n), :] = y.astype(BF16).astype(F32)

        def h_rows(rb, t, m0, n):
            return _ds(H_OFF + ((rb % 2) * NT + t) * (R // 2) + m0 // 2, n // 2)

        def mlp_up(rb, m0, t):
            w = _as_bf16(w1s[_ds(t * (D // 2), D // 2, D // 2), :])
            b = b1f[0:1, _ds(t * 128, 128, 128)]
            h = _gelu(_dot(xn[_ds(rb * R + m0, MU), :], w) + b)
            wa[h_rows(rb, t, m0, MU), :] = pltpu.bitcast(h.astype(BF16), U32)

        def mlp_down(rb, m0, c):
            h = _as_bf16(jnp.concatenate([wa[h_rows(rb, t, m0, MD), :] for t in range(NT)], axis=1))
            y = _dot(h, _as_bf16(w2s[:, c * 128:(c + 1) * 128]))
            b = b2v[pl.ds(c * 128, 128)].astype(F32).reshape(1, 128)
            r0 = rb * R + m0
            wb[_ds(ACC_OFF + c * S + r0, MD), :] = pltpu.bitcast(load_x(r0, MD, c) + (y + b), U32)

        def relayout(g, j, p, half):
            x = wa[_ds(ST_OFF + ((g % 2) * 3 + j) * ST_ROWS + p * 16 * (H // 2), 16 * (H // 2)), :]
            x = x.reshape(8, 2, H // 16, 8, 128)[:, :, half]
            a, b = x[:, 0], x[:, 1]
            even = (a & np.uint32(0xFFFF)) | (b << 16)
            odd = (a >> 16) | (b & np.uint32(0xFFFF0000))
            o0 = group_row0(g) // 2 + p * 8
            for parity, tt in enumerate((_transpose8(even), _transpose8(odd))):
                for i in range(8):
                    h = 2 * (half * 8 + i) + parity
                    wa[_ds(WQ_OFF + (h * 3 + j) * (D // 2) + o0, 8), :] = tt[i]

        start_each(ND, P(x_copy, 0))
        start_each(ND, P(x_copy, 1))
        for cp in small_copies():
            cp.start()
        start_each(NT, w1_copy)
        start_each(ND, P(x_copy, 2))
        start_each(1, w2_copy)
        for j in range(3):
            start_each(1, P(stage_copy, 0, j))
        start_each(ND, P(x_copy, 3))
        for j in range(3):
            start_each(1, P(stage_copy, 1, j))
        start_each(1, wo_copy)

        for rb in range(2):
            x_wait(rb)
            for r0 in range(rb * R, (rb + 1) * R, 128):
                layernorm(r0, 128)
        for cp in small_copies():
            cp.wait()
        b1f[...] = jnp.broadcast_to(b1v[...].astype(F32).reshape(1, F), (8, F))

        def start_body(i, carry):
            for tt in range(TPI):
                w1_copy(i * TPI + tt).wait()
            for tt in range(TPI):
                for rb in range(2):
                    for m0 in range(0, R, MU):
                        mlp_up(rb, m0, i * TPI + tt)
            return carry

        jax.lax.fori_loop(0, NT // TPI, start_body, 0)
        x_wait(2)
        w2_copy().wait()

        def mlp_body(rb, carry):
            @pl.when(rb == 1)
            def _():
                x_wait(3)

            _interleave([P(mlp_down, rb, m0, c) for c in range(ND) for m0 in range(0, R, MD)],
                        [P(layernorm, (rb + 2) * R + r, LN_ROWS) for r in range(0, R, LN_ROWS)])
            for j in range(3):
                stage_copy(rb, j).wait()
            _interleave([P(mlp_up, rb + 2, m0, t) for t in range(NT) for m0 in range(0, R, MU)],
                        [P(relayout, rb, j, p, half) for j in range(3) for p in range(CH // 16)
                         for half in range(H // 16)])

            @pl.when(rb + 2 < NIT)
            def _():
                for j in range(3):
                    stage_copy(rb + 2, j).start()

            return carry

        jax.lax.fori_loop(0, NIT, mlp_body, 0)

        def mlp_tail(i, carry):
            r = (NB - 2) * R + i * MD
            for c in range(ND):
                mlp_down(r // R, r % R, c)
            return carry

        jax.lax.fori_loop(0, 2 * R // MD, mlp_tail, 0)
        wo_copy().wait()

        row = jax.lax.broadcasted_iota(jnp.int32, (G * L, G * L), 0)
        col = jax.lax.broadcasted_iota(jnp.int32, (G * L, G * L), 1)
        row_head = sum(((row >= g * L).astype(jnp.int32) for g in range(1, G)), jnp.zeros_like(row))
        col_head = sum(((col >= g * L).astype(jnp.int32) for g in range(1, G)), jnp.zeros_like(col))
        qi = row - row_head * L
        ki = col - col_head * L
        mask = (row_head == col_head) & ((qi < M) | (qi >= ki))

        def step(s, mem):
            t0 = pl.multiple_of(s * SEG, SEG)
            hx = jnp.concatenate([mem, xn[pl.ds(t0, SEG), :]], axis=0)
            proj = ({}, {}, {})
            sc, e, l, o = {}, {}, {}, {}
            y = [None] * ND

            def heads(g):
                return range(g * G, (g + 1) * G)

            def stack(t, g):
                return jnp.concatenate([t[h] for h in heads(g)], axis=0) if G > 1 else t[g]

            def project(j, g):
                for h in heads(g):
                    w = wa[pl.ds(WQ_OFF + (h * 3 + j) * (D // 2), D // 2), :]
                    proj[j][h] = _dot(hx, _as_bf16(w))

            def scores(g):
                sc[g] = _dot_nt(stack(proj[0], g), stack(proj[1], g).astype(BF16))

            def softmax(g):
                t = jnp.where(mask, sc[g] * scale, np.float32(-1e9))
                e[g] = jnp.exp(t - jnp.max(t, axis=-1, keepdims=True))
                l[g] = jnp.sum(e[g], axis=-1, keepdims=True)

            def pv(g):
                og = _dot(e[g], stack(proj[2], g).astype(BF16)) / l[g]
                for i, h in enumerate(heads(g)):
                    o[h] = og[i * L:(i + 1) * L]

            def out(g):
                for h in heads(g):
                    for c in range(ND):
                        t = _dot(o[h], _as_bf16(wos[h, :, c * 128:(c + 1) * 128]))
                        y[c] = t if y[c] is None else y[c] + t

            stages = {"q": (P(project, 0), 0), "k": (P(project, 1), 0), "v": (P(project, 2), 0),
                      "scores": (scores, LAG_SCORES), "softmax": (softmax, LAG_SCORES),
                      "pv": (pv, LAG_PV), "out": (out, LAG_OUT)}
            for i in range(NG + LAG_OUT):
                for name in SLOT_ORDER:
                    fn, lag = stages[name]
                    if 0 <= i - lag < NG:
                        fn(i - lag)

            yv = jnp.concatenate(y, axis=1)
            res = jnp.concatenate(
                [pltpu.bitcast(wb[_ds(ACC_OFF + c * S + t0, SEG), :], F32) for c in range(ND)],
                axis=1)
            ob[pl.ds(t0, SEG), :] = (res + yv[M:]).astype(BF16)
            out_copy(t0).start()
            return yv[:M]

        def steps(i, mem):
            for u in range(STEP_UNROLL):
                mem = step(i * STEP_UNROLL + u, mem)
            return mem

        jax.lax.fori_loop(0, NSEG // STEP_UNROLL, steps, mem0v[0].astype(F32))
        pltpu.make_async_copy(ob, out_hbm.at[0], sem_out).wait()

    hbm = pl.BlockSpec(memory_space=pl.ANY)
    return pl.pallas_call(
        kernel,
        out_shape=jax.ShapeDtypeStruct(A_x.shape, A_x.dtype),
        in_specs=[hbm] * 10,
        out_specs=hbm,
        scratch_shapes=[
            pltpu.VMEM((WA_ROWS, 128), U32),
            pltpu.VMEM((WB_ROWS, 128), U32),
            pltpu.VMEM((S, D), F32),
            pltpu.VMEM((S, D), BF16),
            pltpu.VMEM((NT * (D // 2), 128), U32),
            pltpu.VMEM((F // 2, D), U32),
            pltpu.VMEM((H, DH // 2, D), U32),
            pltpu.VMEM((8, F), F32),
            pltpu.VMEM((F,), BF16),
            pltpu.VMEM((D,), BF16),
            pltpu.VMEM((1, M, D), BF16),
            pltpu.SemaphoreType.DMA((4,)),
            pltpu.SemaphoreType.DMA((NT // TPI,)),
            pltpu.SemaphoreType.DMA(()),
            pltpu.SemaphoreType.DMA(()),
            pltpu.SemaphoreType.DMA((2, 3)),
            pltpu.SemaphoreType.DMA(()),
            pltpu.SemaphoreType.DMA((3,)),
        ],
        compiler_params=pltpu.CompilerParams(vmem_limit_bytes=110 * 1024 * 1024),
    )(A_x, A_mem0, A_Wq.reshape(D * H, DH), A_Wk.reshape(D * H, DH), A_Wv.reshape(D * H, DH),
      A_Wo, B_w1, B_b1, B_w2, B_b2)
```

```python
import functools
import math

import jax
import jax.numpy as jnp
import numpy as np
import jax.experimental.pallas as pl
import jax.experimental.pallas.tpu as pltpu

F32 = jnp.float32
BF16 = jnp.bfloat16
U32 = jnp.uint32

ROW_BLOCK = 256
UP_ROWS = 64
DOWN_ROWS = 256
LN_ROWS = 32
START_TILES = 4
HEAD_GROUP = 2
STEP_UNROLL = 2
SLOT_ORDER = ("q", "k", "scores", "softmax", "v", "pv", "out")
LAG_SCORES, LAG_PV, LAG_OUT = 1, 3, 4


def _dot(a, b):
    return jnp.dot(a, b, preferred_element_type=F32)


def _dot_nt(a, b):
    return jax.lax.dot_general(a, b, (((1,), (1,)), ((), ())), preferred_element_type=F32)


def _gelu(x):
    c = np.float32(math.sqrt(2.0 / math.pi))
    return 0.5 * x * (1.0 + jnp.tanh(c * (x + np.float32(0.044715) * (x * x * x))))


def _as_bf16(w):
    return pltpu.bitcast(w, BF16)


def _transpose8(e):
    s = jax.lax.broadcasted_iota(jnp.int32, (1, 8, 128), 1)
    for k in (4, 2, 1):
        x = e.reshape(8 // (2 * k), 2, k, 8, 128)
        a = x[:, 0].reshape(4, 8, 128)
        b = x[:, 1].reshape(4, 8, 128)
        keep = (s & k) == 0
        na = jnp.where(keep, a, pltpu.roll(b, k, 1)).reshape(8 // (2 * k), 1, k, 8, 128)
        nb = jnp.where(keep, pltpu.roll(a, 8 - k, 1), b).reshape(8 // (2 * k), 1, k, 8, 128)
        e = jnp.concatenate([na, nb], axis=1).reshape(8, 8, 128)
    return e


def _ds(start, size, align=8):
    if isinstance(start, int):
        return pl.ds(start, size)
    return pl.ds(pl.multiple_of(start, align), size)


def _interleave(work, pieces):
    done = 0
    for i, w in enumerate(work):
        w()
        upto = min(((i + 1) * len(pieces)) // max(len(work) - 1, 1), len(pieces))
        while done < upto:
            pieces[done]()
            done += 1


@functools.partial(jax.jit, static_argnames=("A_seg_len",))
def pallas_parallel_sum__memory_aug_recurrent_mem_tr__dense_activation_gelu__prompt_kernel(
    A_x: jax.Array,
    A_mem0: jax.Array,
    A_Wq: jax.Array,
    A_Wk: jax.Array,
    A_Wv: jax.Array,
    A_Wo: jax.Array,
    A_seg_len: int,
    B_x: jax.Array,
    B_w1: jax.Array,
    B_b1: jax.Array,
    B_w2: jax.Array,
    B_b2: jax.Array,
):
    del B_x
    _, S, D = A_x.shape
    M = A_mem0.shape[1]
    _, H, DH = A_Wq.shape
    F = B_w1.shape[1]
    SEG = int(A_seg_len)
    NSEG = S // SEG
    L = M + SEG
    scale = np.float32(DH ** (-0.5))

    R, MU, MD, TPI, G = ROW_BLOCK, UP_ROWS, DOWN_ROWS, START_TILES, HEAD_GROUP
    NB = S // R
    NIT = NB - 2
    ND = D // 128
    NT = F // 128
    NG = H // G
    CH = -(-D // (16 * NIT)) * 16
    assert DH == 128 and H % 16 == 0 and H % G == 0 and G * L <= 128
    assert M % 8 == 0 and SEG % 16 == 0 and NSEG % STEP_UNROLL == 0
    assert S % R == 0 and NB >= 4 and NT % TPI == 0 and D % 128 == 0 and F % 128 == 0

    H_OFF = 0
    WQ_OFF = H_OFF + 2 * NT * (R // 2)
    WA_ROWS = WQ_OFF + H * 3 * (D // 2)

    def kernel(x_hbm, mem0_hbm, wq_hbm, wk_hbm, wv_hbm, wo_hbm, w1_hbm, b1_hbm, w2_hbm, b2_hbm,
               out_hbm,
               wa, acc, xn, xs, stage, ob, w1s, w2s, wos, b1f, b1v, b2v, mem0v,
               sem_x, sem_w1, sem_w2, sem_wo, sem_st, sem_out, sem_small):
        w_hbm = (wq_hbm, wk_hbm, wv_hbm)
        P = functools.partial

        XG = ((0, R), (R, R), (2 * R, R), (3 * R, S - 3 * R))

        def x_copy(g, _=None):
            r0, n = XG[g]
            return pltpu.make_async_copy(
                x_hbm.at[0, pl.ds(r0, n), :], xs.at[pl.ds(r0, n), :], sem_x.at[g])

        def w1_copy(t):
            return pltpu.make_async_copy(
                w1_hbm.at[:, _ds(t * 128, 128, 128)], w1s.at[t], sem_w1.at[t // TPI])

        def small_copies():
            return (pltpu.make_async_copy(b1_hbm, b1v, sem_small.at[0]),
                    pltpu.make_async_copy(b2_hbm, b2v, sem_small.at[1]),
                    pltpu.make_async_copy(mem0_hbm, mem0v, sem_small.at[2]))

        def w2_copy(c):
            return pltpu.make_async_copy(w2_hbm.at[:, _ds(c * 128, 128, 128)], w2s.at[c], sem_w2)

        def wo_copy(c):
            return pltpu.make_async_copy(wo_hbm.at[:, :, _ds(c * 128, 128, 128)], wos.at[c], sem_wo)

        def group_row0(g):
            if isinstance(g, int):
                return min(g * CH, D - CH)
            return pl.multiple_of(jnp.minimum(g * CH, D - CH), 16)

        def stage_copy(g, j, _=None):
            slot = g % 2
            return pltpu.make_async_copy(
                w_hbm[j].at[pl.ds(group_row0(g), CH)], stage.at[slot, j], sem_st.at[slot, j])

        def out_copy(t0):
            return pltpu.make_async_copy(
                ob.at[pl.ds(t0, SEG), :], out_hbm.at[0, pl.ds(t0, SEG), :], sem_out)

        def start_each(n, make_copy):
            def body(i, carry):
                make_copy(i).start()
                return carry
            jax.lax.fori_loop(0, n, body, 0)

        def layernorm(r0, n):
            x = xs[_ds(r0, n, 16), :].astype(F32)
            mean = jnp.mean(x, axis=-1, keepdims=True)
            xc = x - mean
            var = jnp.mean(xc * xc, axis=-1, keepdims=True)
            y = (xc * jax.lax.rsqrt(var + np.float32(1e-5))).astype(BF16).astype(F32)
            xn[_ds(r0, n), :] = y

        def h_rows(rb, t, m0, n):
            return _ds(H_OFF + ((rb % 2) * NT + t) * (R // 2) + m0 // 2, n // 2)

        def mlp_up(rb, m0, t):
            b = b1f[0:1, _ds(t * 128, 128, 128)]
            h = _gelu(_dot(xn[_ds(rb * R + m0, MU), :], w1s[t]) + b)
            wa[h_rows(rb, t, m0, MU), :] = pltpu.bitcast(h.astype(BF16), U32)

        def mlp_down(rb, m0, c):
            h = _as_bf16(jnp.concatenate([wa[h_rows(rb, t, m0, MD), :] for t in range(NT)], axis=1))
            y = _dot(h, w2s[c])
            b = b2v[pl.ds(c * 128, 128)].astype(F32).reshape(1, 128)
            r0 = rb * R + m0
            x = xs[_ds(r0, MD, 16), c * 128:(c + 1) * 128].astype(F32)
            acc[_ds(r0, MD), c * 128:(c + 1) * 128] = x + (y + b)
            xs[S:S + 16, 0:128] = jnp.zeros((16, 128), BF16)

        def relayout(g, j, p, half, parity):
            x = stage[g % 2, j, p * 16:(p + 1) * 16, half * 16:(half + 1) * 16, :]
            x = pltpu.bitcast(x.reshape(16 * 16, 128), U32).reshape(8, 2, 8, 128)
            a, b = x[:, 0], x[:, 1]
            if parity == 0:
                w = (a & np.uint32(0xFFFF)) | (b << 16)
            else:
                w = (a >> 16) | (b & np.uint32(0xFFFF0000))
            o0 = group_row0(g) // 2 + p * 8
            tt = _transpose8(w)
            for i in range(8):
                h = 2 * (half * 8 + i) + parity
                wa[_ds(WQ_OFF + (h * 3 + j) * (D // 2) + o0, 8), :] = tt[i]

        start_each(1, P(x_copy, 0))
        start_each(1, P(x_copy, 1))
        for cp in small_copies():
            cp.start()
        start_each(NT, w1_copy)
        start_each(1, P(x_copy, 2))
        start_each(ND, w2_copy)
        for j in range(3):
            start_each(1, P(stage_copy, 0, j))
        start_each(1, P(x_copy, 3))
        for j in range(3):
            start_each(1, P(stage_copy, 1, j))
        start_each(ND, wo_copy)

        for rb in range(2):
            x_copy(rb).wait()
            for r0 in range(rb * R, (rb + 1) * R, 128):
                layernorm(r0, 128)
        for cp in small_copies():
            cp.wait()
        b1f[...] = jnp.broadcast_to(b1v[...].astype(F32).reshape(1, F), (8, F))

        def start_body(i, carry):
            for tt in range(TPI):
                w1_copy(i * TPI + tt).wait()
            for tt in range(TPI):
                for rb in range(2):
                    for m0 in range(0, R, MU):
                        mlp_up(rb, m0, i * TPI + tt)
            return carry

        jax.lax.fori_loop(0, NT // TPI, start_body, 0)
        x_copy(2).wait()
        for c in range(ND):
            w2_copy(c).wait()

        def mlp_body(rb, carry):
            @pl.when(rb == 1)
            def _():
                x_copy(3).wait()

            _interleave([P(mlp_down, rb, m0, c) for c in range(ND) for m0 in range(0, R, MD)],
                        [P(layernorm, (rb + 2) * R + r, LN_ROWS) for r in range(0, R, LN_ROWS)])
            for j in range(3):
                stage_copy(rb, j).wait()
            _interleave([P(mlp_up, rb + 2, m0, t) for t in range(NT) for m0 in range(0, R, MU)],
                        [P(relayout, rb, j, p, half, par) for j in range(3)
                         for p in range(CH // 16) for half in range(H // 16) for par in range(2)])

            @pl.when(rb + 2 < NIT)
            def _():
                for j in range(3):
                    stage_copy(rb + 2, j).start()

            return carry

        jax.lax.fori_loop(0, NIT, mlp_body, 0)

        def mlp_tail(i, carry):
            r = (NB - 2) * R + i * MD
            for c in range(ND):
                mlp_down(r // R, r % R, c)
            return carry

        jax.lax.fori_loop(0, 2 * R // MD, mlp_tail, 0)
        for c in range(ND):
            wo_copy(c).wait()

        row = jax.lax.broadcasted_iota(jnp.int32, (G * L, G * L), 0)
        col = jax.lax.broadcasted_iota(jnp.int32, (G * L, G * L), 1)
        row_head = sum(((row >= g * L).astype(jnp.int32) for g in range(1, G)), jnp.zeros_like(row))
        col_head = sum(((col >= g * L).astype(jnp.int32) for g in range(1, G)), jnp.zeros_like(col))
        qi = row - row_head * L
        ki = col - col_head * L
        same_head = row_head == col_head
        mask = same_head & ((qi < M) | (qi >= ki))
        fill = jnp.where(same_head, np.float32(-1e9), np.float32(-np.inf))

        def step(s, mem):
            t0 = pl.multiple_of(s * SEG, SEG)
            hx = jnp.concatenate([mem, xn[pl.ds(t0, SEG), :]], axis=0)
            proj = ({}, {}, {})
            sc, e, l, o = {}, {}, {}, {}
            y = [None] * ND

            def heads(g):
                return range(g * G, (g + 1) * G)

            def stack(t, g):
                return jnp.concatenate([t[h] for h in heads(g)], axis=0) if G > 1 else t[g]

            def project(j, g):
                for h in heads(g):
                    w = wa[pl.ds(WQ_OFF + (h * 3 + j) * (D // 2), D // 2), :]
                    proj[j][h] = _dot(hx, _as_bf16(w))

            def scores(g):
                sc[g] = _dot_nt(stack(proj[0], g), stack(proj[1], g).astype(BF16))

            def softmax(g):
                t = jnp.where(mask, sc[g] * scale, fill)
                e[g] = jnp.exp(t - jnp.max(t, axis=-1, keepdims=True))
                l[g] = jnp.sum(e[g], axis=-1, keepdims=True)

            def pv(g):
                og = _dot(e[g], stack(proj[2], g).astype(BF16)) / l[g]
                for i, h in enumerate(heads(g)):
                    o[h] = og[i * L:(i + 1) * L]

            def out(g):
                for h in heads(g):
                    for c in range(ND):
                        t = _dot(o[h], wos[c, h])
                        y[c] = t if y[c] is None else y[c] + t

            stages = {"q": (P(project, 0), 0), "k": (P(project, 1), 0), "v": (P(project, 2), 0),
                      "scores": (scores, LAG_SCORES), "softmax": (softmax, LAG_SCORES),
                      "pv": (pv, LAG_PV), "out": (out, LAG_OUT)}
            for i in range(NG + LAG_OUT):
                for name in SLOT_ORDER:
                    fn, lag = stages[name]
                    if 0 <= i - lag < NG:
                        fn(i - lag)

            yv = jnp.concatenate(y, axis=1)
            res = acc[pl.ds(t0, SEG), :]
            ob[pl.ds(t0, SEG), :] = (res + yv[M:]).astype(BF16)
            out_copy(t0).start()
            return yv[:M]

        def steps(i, mem):
            for u in range(STEP_UNROLL):
                mem = step(i * STEP_UNROLL + u, mem)
            return mem

        jax.lax.fori_loop(0, NSEG // STEP_UNROLL, steps, mem0v[0].astype(F32))
        pltpu.make_async_copy(ob, out_hbm.at[0], sem_out).wait()

    hbm = pl.BlockSpec(memory_space=pl.ANY)
    return pl.pallas_call(
        kernel,
        out_shape=jax.ShapeDtypeStruct(A_x.shape, A_x.dtype),
        in_specs=[hbm] * 10,
        out_specs=hbm,
        scratch_shapes=[
            pltpu.VMEM((WA_ROWS, 128), U32),
            pltpu.VMEM((S, D), F32),
            pltpu.VMEM((S, D), F32),
            pltpu.VMEM((S + 16, D), BF16),
            pltpu.VMEM((2, 3, CH, H, DH), BF16),
            pltpu.VMEM((S, D), BF16),
            pltpu.VMEM((NT, D, 128), BF16),
            pltpu.VMEM((ND, F, 128), BF16),
            pltpu.VMEM((ND, H, DH, 128), BF16),
            pltpu.VMEM((8, F), F32),
            pltpu.VMEM((F,), BF16),
            pltpu.VMEM((D,), BF16),
            pltpu.VMEM((1, M, D), BF16),
            pltpu.SemaphoreType.DMA((4,)),
            pltpu.SemaphoreType.DMA((NT // TPI,)),
            pltpu.SemaphoreType.DMA(()),
            pltpu.SemaphoreType.DMA(()),
            pltpu.SemaphoreType.DMA((2, 3)),
            pltpu.SemaphoreType.DMA(()),
            pltpu.SemaphoreType.DMA((3,)),
        ],
        compiler_params=pltpu.CompilerParams(vmem_limit_bytes=110 * 1024 * 1024),
    )(A_x, A_mem0, A_Wq, A_Wk, A_Wv, A_Wo, B_w1, B_b1, B_w2, B_b2)
```
